```python
import jax
import jax.numpy as jnp

def _softmax(x, axis=-1):
    return jax.nn.softmax(x, axis=axis)

def _gelu(x):
    return jax.nn.gelu(x, approximate=True)

def _silu(x):
    return jax.nn.silu(x)

def _sigmoid(x):
    return jax.nn.sigmoid(x)

def _layernorm(x, axis=-1, eps=1e-05):
    m = jnp.mean(x, axis=axis, keepdims=True)
    v = jnp.var(x, axis=axis, keepdims=True)
    return (x - m) / jnp.sqrt(v + eps)

def _scatter_add(tgt, idx, src, axis=0):
    return tgt.at[idx].add(src)

def _segment_sum(src, seg, n):
    return jax.ops.segment_sum(src, seg, n)

class _Rng:

    def __init__(self, key):
        self._k = key

    def _next(self):
        self._k, sub = jax.random.split(self._k)
        return sub

    def normal(self, shape):
        return jax.random.normal(self._next(), shape, dtype=jnp.bfloat16)

    def randint(self, lo, hi, shape):
        return jax.random.randint(self._next(), shape, lo, hi, dtype=jnp.int32)

    def uniform(self, shape, lo=0.0, hi=1.0):
        return jax.random.uniform(self._next(), shape, jnp.bfloat16, lo, hi)

    def permutation(self, n):
        return jax.random.permutation(self._next(), n)
kernel_name = 'recurrent_scan__memory_aug_recurrent_mem_tr__mixer_s_mlp__prompt'

def setup_inputs():
    _rng = _Rng(jax.random.key(int.from_bytes(__import__("os").urandom(4), "little")))
    _w = lambda a: (lambda t: t.astype(jnp.bfloat16) if jnp.issubdtype(t.dtype, jnp.floating) else t)(jnp.asarray(a))

    def _A_setup():
        B, S, Dm = (1, 2048, 1024)
        H, Dh = (32, 128)
        M, seg = (8, 32)
        seg = min(seg, S)
        S = S // seg * seg
        return {'x': _w((lambda *s: _rng.normal(s) * 0.05)(B, S, Dm)), 'mem0': _w((lambda *s: _rng.normal(s) * 0.05)(B, M, Dm)), 'Wq': _w((lambda *s: _rng.normal(s) * 0.05)(Dm, H, Dh) * Dm ** (-0.5)), 'Wk': _w((lambda *s: _rng.normal(s) * 0.05)(Dm, H, Dh) * Dm ** (-0.5)), 'Wv': _w((lambda *s: _rng.normal(s) * 0.05)(Dm, H, Dh) * Dm ** (-0.5)), 'Wo': _w((lambda *s: _rng.normal(s) * 0.05)(H, Dh, Dm) * (H * Dh) ** (-0.5)), 'seg_len': seg}
    _A_in = _A_setup()

    def _B_setup():
        B, S, D, F = (1, 2048, 1024, 3584)
        return {'x': _w((lambda *s: _rng.normal(s) * 0.05)(B, S, D)), 'w1': _w((lambda *s: _rng.normal(s) * 0.05)(D, D) * D ** (-0.5)), 'w2': _w((lambda *s: _rng.normal(s) * 0.05)(D, D) * D ** (-0.5)), 'w3': _w((lambda *s: _rng.normal(s) * 0.05)(D, F) * D ** (-0.5)), 'w4': _w((lambda *s: _rng.normal(s) * 0.05)(F, D) * F ** (-0.5))}
    _B_in = _B_setup()
    return {'A_x': _A_in['x'], 'A_mem0': _A_in['mem0'], 'A_Wq': _A_in['Wq'], 'A_Wk': _A_in['Wk'], 'A_Wv': _A_in['Wv'], 'A_Wo': _A_in['Wo'], 'A_seg_len': _A_in['seg_len'], 'B_x': _B_in['x'], 'B_w1': _B_in['w1'], 'B_w2': _B_in['w2'], 'B_w3': _B_in['w3'], 'B_w4': _B_in['w4']}

def reference(A_x, A_mem0, A_Wq, A_Wk, A_Wv, A_Wo, A_seg_len, B_x, B_w1, B_w2, B_w3, B_w4):

    def _A_ref(x, mem0, Wq, Wk, Wv, Wo, seg_len):
        B, S, Dm = x.shape
        H, Dh = (Wq.shape[1], Wq.shape[2])
        M = mem0.shape[1]
        scale = Dh ** (-0.5)
        n_seg = S // seg_len
        L = M + seg_len
        idx = jnp.arange(L)
        mask = (idx[:, None] < M) | (idx[:, None] >= idx[None, :])
        mem = mem0
        outs = []
        for s in range(n_seg):
            xs = x[:, s * seg_len:(s + 1) * seg_len, :].copy()
            h = jnp.concatenate([mem, xs], axis=1)
            q = jnp.einsum('btd,dhe->bhte', h, Wq)
            k = jnp.einsum('btd,dhe->bhte', h, Wk)
            v = jnp.einsum('btd,dhe->bhte', h, Wv)
            scores = jnp.einsum('bhqe,bhke->bhqk', q, k) * scale
            scores = jnp.where(mask[None, None], scores, -1000000000.0)
            p = _softmax(scores, axis=-1)
            o = jnp.einsum('bhqk,bhke->bhqe', p, v)
            o = jnp.einsum('bhte,hed->btd', o, Wo)
            mem = o[:, :M, :].copy()
            outs.append(o[:, M:, :])
        return jnp.concatenate(outs, axis=1)

    def _B_ref(x, w1, w2, w3, w4):
        B, S, D = x.shape
        h = _gelu(_layernorm(x, axis=-1) @ w1)
        c = D // 4
        g0 = jnp.pad(h[:, :, 0 * c:1 * c], ((0, 0), (1, 0), (0, 0)))[:, :S, :]
        g1 = jnp.pad(h[:, :, 1 * c:2 * c], ((0, 0), (0, 1), (0, 0)))[:, 1:, :]
        g2 = jnp.pad(h[:, :, 2 * c:3 * c], ((0, 0), (2, 0), (0, 0)))[:, :S, :]
        g3 = jnp.pad(h[:, :, 3 * c:], ((0, 0), (0, 2), (0, 0)))[:, 2:, :]
        hs = jnp.concatenate([g0, g1, g2, g3], axis=-1) @ w2
        x1 = x + hs
        h2 = _gelu(_layernorm(x1, axis=-1) @ w3) @ w4
        return x1 + h2
    x = A_x
    xn = _layernorm(x, axis=-1)
    s = _A_ref(xn, A_mem0, A_Wq, A_Wk, A_Wv, A_Wo, A_seg_len)
    g = _silu(_B_ref(xn, B_w1, B_w2, B_w3, B_w4))
    return x + s * g
```

```python
import functools

import jax
import jax.numpy as jnp
import jax.experimental.pallas as pl
import jax.experimental.pallas.tpu as pltpu

F32 = jnp.float32
BF16 = jnp.bfloat16
U32 = jnp.uint32

LANES = 128
HALO = 8
ROWS = 256

_NN = (((1,), (0,)), ((), ()))
_NT = (((1,), (1,)), ((), ()))


def _dot(a, b, dims=_NN):
    return jax.lax.dot_general(a, b, dims, preferred_element_type=F32)


def _layernorm(x, eps=1e-5):
    d = x - jnp.mean(x, axis=-1, keepdims=True)
    return d * jax.lax.rsqrt(jnp.mean(d * d, axis=-1, keepdims=True) + eps)


def _gelu(x):
    return jax.nn.gelu(x, approximate=True)


def _kernel(
    x_hbm, mem_ref, wq_hbm, wk_hbm, wv_hbm, wo_hbm, w1_hbm, w2_hbm, w3_hbm, w4_hbm,
    out_hbm,
    x_v, xn_v, h_v, g_v, out_v, w1_v, w2_v, w3_v, w4_v, stage_v, wqkv_v, wo_v,
    x_sems, w_sems, wo_sems, out_sem,
    *, seg,
):
    S, D = x_v.shape
    H, E = stage_v.shape[2:]
    F = w3_v.shape[1]
    M = mem_ref.shape[0]
    L = M + seg
    n_blk = S // ROWS
    n_col = D // LANES

    def x_copy(i):
        rows = pl.ds(i * ROWS, ROWS)
        return pltpu.make_async_copy(x_hbm.at[rows], x_v.at[rows], x_sems.at[i])

    w_copies = [
        pltpu.make_async_copy(src, dst, w_sems.at[i])
        for i, (src, dst) in enumerate((
            (w1_hbm, w1_v), (w2_hbm, w2_v), (w3_hbm, w3_v), (w4_hbm, w4_v),
            (wq_hbm, stage_v.at[0]), (wk_hbm, stage_v.at[1]), (wv_hbm, stage_v.at[2]),
        ))
    ]
    wo_bf = wo_v.bitcast(BF16)
    wo_copies = [
        pltpu.make_async_copy(
            wo_hbm.at[:, pl.ds(j * LANES, LANES)], wo_bf.at[j], wo_sems.at[j])
        for j in range(n_col)
    ]
    x_copy(0).start()
    w_copies[0].start()
    for i in range(1, n_blk):
        x_copy(i).start()
    for c in w_copies[1:] + wo_copies:
        c.start()

    h_v[pl.ds(0, HALO), :] = jnp.zeros((HALO, D), F32)
    h_v[pl.ds(HALO + S, HALO), :] = jnp.zeros((HALO, D), F32)
    w_copies[0].wait()

    def stage1(i, carry):
        x_copy(i).wait()
        r0 = pl.multiple_of(i * ROWS, ROWS)
        xn = _layernorm(x_v[pl.ds(r0, ROWS), :].astype(F32))
        xn_v[pl.ds(r0, ROWS), :] = xn
        h = _gelu(_dot(_layernorm(xn).astype(BF16), w1_v[...]))
        h_v[pl.ds(r0 + HALO, ROWS), :] = h
        return carry

    jax.lax.fori_loop(0, n_blk, stage1, 0)

    for c in w_copies[1:4]:
        c.wait()
    C = D // 4
    FC = 512

    def stage2(i, carry):
        r0 = pl.multiple_of(i * ROWS, ROWS)
        parts = []
        for c, shift in enumerate((-1, 1, -2, 2)):
            win = h_v[pl.ds(r0, ROWS + 2 * HALO), pl.ds(c * C, C)]
            parts.append(win[HALO + shift:HALO + shift + ROWS].astype(BF16))
        hs = _dot(jnp.concatenate(parts, axis=-1), w2_v[...])
        x1 = xn_v[pl.ds(r0, ROWS), :] + hs
        ln = _layernorm(x1).astype(BF16)
        acc = x1
        for f in range(F // FC):
            u = _gelu(_dot(ln, w3_v[:, pl.ds(f * FC, FC)])).astype(BF16)
            acc = acc + _dot(u, w4_v[pl.ds(f * FC, FC), :])
        g_v[pl.ds(r0, ROWS), :] = jax.nn.silu(acc)
        return carry

    jax.lax.fori_loop(0, n_blk, stage2, 0)

    DC = 64
    for t in range(3):
        w_copies[4 + t].wait()

        def relayout(i, carry, t=t):
            w = stage_v[t, pl.ds(pl.multiple_of(i * DC, DC), DC), :, :]
            w = pltpu.bitcast(jnp.swapaxes(w, 0, 1), U32)
            r0 = pl.multiple_of(i * (DC // 2), DC // 2)
            wqkv_v[:, pl.ds(r0, DC // 2), pl.ds(t * E, E)] = w
            return carry

        jax.lax.fori_loop(0, D // DC, relayout, 0)
    for c in wo_copies:
        c.wait()

    scale = E ** -0.5
    qi = jax.lax.broadcasted_iota(jnp.int32, (L, L), 0)
    ki = jax.lax.broadcasted_iota(jnp.int32, (L, L), 1)
    mask = (qi < M) | (qi >= ki)

    def step(s, mem):
        r0 = pl.multiple_of(s * seg, seg)
        rows = pl.ds(r0, seg)
        hin = jnp.concatenate([mem, xn_v[rows, :]], axis=0)
        qkv, prob, outs = {}, {}, {}
        for it in range(H + 3):
            if it < H:
                qkv[it] = _dot(hin, pltpu.bitcast(wqkv_v[it], BF16))
            hd = it - 1
            if 0 <= hd < H:
                sc = _dot(qkv[hd][:, :E], qkv[hd][:, E:2 * E], _NT) * scale
                sc = jnp.where(mask, sc, -1e9)
                e = jnp.exp(sc - jnp.max(sc, axis=-1, keepdims=True))
                prob[hd] = (e, jnp.sum(e, axis=-1, keepdims=True))
            hd = it - 3
            if 0 <= hd < H:
                e, l = prob.pop(hd)
                outs[hd] = _dot(e, qkv.pop(hd)[:, 2 * E:]) / l
        o = jnp.concatenate([outs[hd] for hd in range(H)], axis=-1)
        o = jnp.concatenate(
            [_dot(o, pltpu.bitcast(wo_v[j], BF16)) for j in range(n_col)], axis=-1)
        res = x_v[rows, :].astype(F32) + o[M:] * g_v[rows, :]
        out_v[rows, :] = res.astype(out_v.dtype)
        pltpu.make_async_copy(out_v.at[rows], out_hbm.at[rows], out_sem).start()
        return o[:M]

    jax.lax.fori_loop(0, S // seg, step, mem_ref[...].astype(F32))
    pltpu.make_async_copy(out_v, out_hbm, out_sem).wait()


@functools.partial(jax.jit, static_argnames=("A_seg_len",))
def pallas_recurrent_scan__memory_aug_recurrent_mem_tr__mixer_s_mlp__prompt_kernel(
    A_x: jax.Array,
    A_mem0: jax.Array,
    A_Wq: jax.Array,
    A_Wk: jax.Array,
    A_Wv: jax.Array,
    A_Wo: jax.Array,
    A_seg_len: int,
    B_x: jax.Array,
    B_w1: jax.Array,
    B_w2: jax.Array,
    B_w3: jax.Array,
    B_w4: jax.Array,
):
    del B_x
    B, S, D = A_x.shape
    _, H, E = A_Wq.shape
    M = A_mem0.shape[1]
    F = B_w3.shape[1]
    seg = int(A_seg_len)
    assert B == 1 and S % ROWS == 0 and S % seg == 0 and E == LANES

    hbm = pl.BlockSpec(memory_space=pl.ANY)
    out = pl.pallas_call(
        functools.partial(_kernel, seg=seg),
        out_shape=jax.ShapeDtypeStruct((S, D), A_x.dtype),
        in_specs=[hbm, pl.BlockSpec(memory_space=pltpu.VMEM)] + [hbm] * 8,
        out_specs=hbm,
        scratch_shapes=[
            pltpu.VMEM((S, D), BF16),
            pltpu.VMEM((S, D), F32),
            pltpu.VMEM((S + 2 * HALO, D), F32),
            pltpu.VMEM((S, D), F32),
            pltpu.VMEM((S, D), A_x.dtype),
            pltpu.VMEM((D, D), BF16),
            pltpu.VMEM((D, D), BF16),
            pltpu.VMEM((D, F), BF16),
            pltpu.VMEM((F, D), BF16),
            pltpu.VMEM((3, D, H, E), BF16),
            pltpu.VMEM((H, D // 2, 3 * E), U32),
            pltpu.VMEM((D // LANES, H * E // 2, LANES), U32),
            pltpu.SemaphoreType.DMA((S // ROWS,)),
            pltpu.SemaphoreType.DMA((7,)),
            pltpu.SemaphoreType.DMA((D // LANES,)),
            pltpu.SemaphoreType.DMA(()),
        ],
        compiler_params=pltpu.CompilerParams(vmem_limit_bytes=120 * 1024 * 1024),
    )(
        A_x.reshape(S, D), A_mem0.reshape(M, D), A_Wq, A_Wk, A_Wv,
        A_Wo.reshape(H * E, D), B_w1, B_w2, B_w3, B_w4,
    )
    return out.reshape(B, S, D)
```

```python
import functools

import jax
import jax.numpy as jnp
import jax.experimental.pallas as pl
import jax.experimental.pallas.tpu as pltpu

F32 = jnp.float32
BF16 = jnp.bfloat16
U32 = jnp.uint32

LANES = 128
HALO = 8
ROWS1 = 256
ROWS = 256
PLAIN = 2
FC = 512
UNROLL = 2
HSPLIT = 24
KSPLIT = 2
LAG_S = 1
LAG_P = 3

_NN = (((1,), (0,)), ((), ()))
_NT = (((1,), (1,)), ((), ()))


def _dot(a, b, dims=_NN):
    return jax.lax.dot_general(a, b, dims, preferred_element_type=F32)


def _dq(a, b):
    return jax.lax.dot_general(a, b, _NN, preferred_element_type=F32)
def _ds(a, b):
    return jax.lax.dot_general(a, b, _NT, preferred_element_type=F32)
def _dp(a, b):
    return jax.lax.dot_general(a, b, _NN, preferred_element_type=F32)
def _d1(a, b):
    return jax.lax.dot_general(a, b, _NN, preferred_element_type=F32)
def _d2(a, b):
    return jax.lax.dot_general(a, b, _NN, preferred_element_type=F32)
def _d0(a, b):
    return jax.lax.dot_general(a, b, _NN, preferred_element_type=F32)


def _layernorm(x, eps=1e-5):
    d = x - jnp.mean(x, axis=-1, keepdims=True)
    return d * jax.lax.rsqrt(jnp.mean(d * d, axis=-1, keepdims=True) + eps)


def _recip(x):
    r = pl.reciprocal(x, approx=True)
    return r * (2.0 - x * r)


def _gelu(x):
    return jax.nn.gelu(x, approximate=True)


def _kernel(
    x_hbm, mem_ref, wq_hbm, wk_hbm, wv_hbm, wo_hbm, w1_hbm, w2_hbm, w3_hbm, w4_hbm,
    out_hbm,
    x_v, xn_v, ln_v, h_v, g_v, out_v, w1_v, w2_v, w3_v, w4_v, stage_v, tmp_v, wqkv_v, wo_v,
    x_sems, w_sems, wo_sems, out_sem,
    *, seg,
):
    S, D = x_v.shape
    H, E = wqkv_v.shape[0], LANES
    F = w3_v.shape[1]
    M = mem_ref.shape[0]
    L = M + seg
    n_col = D // LANES

    n1 = S // ROWS1

    def x_copy(i):
        rows = pl.ds(i * ROWS1, ROWS1)
        return pltpu.make_async_copy(x_hbm.at[rows], x_v.at[rows], x_sems.at[i])

    stage_bf = stage_v.bitcast(BF16)
    w_copies = [
        pltpu.make_async_copy(src, dst, w_sems.at[i])
        for i, (src, dst) in enumerate((
            (w1_hbm, w1_v), (w2_hbm, w2_v), (w3_hbm, w3_v), (w4_hbm, w4_v),
            (wq_hbm, stage_bf.at[0]), (wk_hbm, stage_bf.at[1]), (wv_hbm, stage_bf.at[2]),
        ))
    ]
    wo_bf = wo_v.bitcast(BF16)
    wo_copies = [
        pltpu.make_async_copy(
            wo_hbm.at[:, pl.ds(j * LANES, LANES)], wo_bf.at[j], wo_sems.at[j])
        for j in range(n_col)
    ]
    x_copy(0).start()
    w_copies[0].start()
    x_copy(1).start()

    h_v[pl.ds(0, HALO), :] = jnp.zeros((HALO, D), F32)
    h_v[pl.ds(HALO + S, HALO), :] = jnp.zeros((HALO, D), F32)

    def norm(i):
        r0 = pl.multiple_of(i * ROWS1, ROWS1)
        xn = _layernorm(x_v[pl.ds(r0, ROWS1), :].astype(F32))
        xn_v[pl.ds(r0, ROWS1), :] = xn
        ln_v[i % 2] = _layernorm(xn).astype(BF16)

    def project(i):
        r0 = pl.multiple_of(i * ROWS1, ROWS1)
        h_v[pl.ds(r0 + HALO, ROWS1), :] = _gelu(_dot(ln_v[i % 2], w1_v[...]))

    with jax.named_scope('p_wait1'):
        x_copy(0).wait()
        norm(0)
        w_copies[0].wait()
    for i in range(2, n1):
        x_copy(i).start()
    for c in w_copies[1:4]:
        c.start()

    def stage1(i, carry):
        x_copy(i + 1).wait()
        project(i)
        norm(i + 1)
        return carry

    with jax.named_scope('p_stage1'):
        jax.lax.fori_loop(0, n1 - 1, stage1, 0)
        project(n1 - 1)

    with jax.named_scope('p_wait234'):
        for c in w_copies[1:4]:
            c.wait()
    for c in w_copies[4:] + wo_copies:
        c.start()
    C = D // 4
    n2 = S // ROWS
    DC = 64

    def stage2(i, carry):
        r0 = pl.multiple_of(i * ROWS, ROWS)
        parts = []
        for c, shift in enumerate((-1, 1, -2, 2)):
            win = h_v[pl.ds(r0, ROWS + 2 * HALO), pl.ds(c * C, C)]
            parts.append(win[HALO + shift:HALO + shift + ROWS].astype(BF16))
        hs = _dot(jnp.concatenate(parts, axis=-1), w2_v[...])
        x1 = xn_v[pl.ds(r0, ROWS), :] + hs
        ln = _layernorm(x1).astype(BF16)
        acc = x1
        for f in range(F // FC):
            u = _gelu(_dot(ln, w3_v[:, pl.ds(f * FC, FC)])).astype(BF16)
            acc = acc + _dot(u, w4_v[pl.ds(f * FC, FC), :])
        g_v[pl.ds(r0, ROWS), :] = jax.nn.silu(acc)
        return carry

    with jax.named_scope('p_stage2'):
        jax.lax.fori_loop(0, n2, stage2, 0)
    with jax.named_scope('p_waitA'):
        for c in w_copies[4:] + wo_copies:
            c.wait()

    def relayout(c, carry):
        base = pl.multiple_of(c * (DC * H // 2), DC * H // 2)
        dst = pl.ds(pl.multiple_of(c * (DC // 2), DC // 2), DC // 2)
        G = H // 8
        for t in range(3):
            for j0 in range(4):
                tmp_v[t, j0] = stage_v[t, pl.ds(base + j0, DC * G, stride=4), :]
            for j0 in range(4):
                for j1 in range(G):
                    w = tmp_v[t, j0, pl.ds(j1, DC, stride=G), :]
                    for half, bits in enumerate((w, w >> 16)):
                        wqkv_v[2 * (4 * j1 + j0) + half, dst, pl.ds(t * E, E)] = pltpu.bitcast(
                            bits.astype(jnp.uint16), U32)
        return carry

    with jax.named_scope('p_relayout'):
        jax.lax.fori_loop(0, D // DC, relayout, 0)

    scale = E ** -0.5
    qi = jax.lax.broadcasted_iota(jnp.int32, (L, L), 0)
    ki = jax.lax.broadcasted_iota(jnp.int32, (L, L), 1)
    mask = (qi < M) | (qi >= ki)
    K1 = HSPLIT * E // 2

    def step(s, mem):
        r0 = pl.multiple_of(s * seg, seg)
        rows = pl.ds(r0, seg)
        hin = jnp.concatenate([mem, xn_v[rows, :]], axis=0)
        qkv, prob, outs = {}, {}, {}

        def scores(hd):
            sc = _ds(qkv[hd][:, :E], qkv[hd][:, E:2 * E]) * scale
            sc = jnp.where(mask, sc, -1e9)
            e = jnp.exp(sc - jnp.max(sc, axis=-1, keepdims=True))
            prob[hd] = e * _recip(jnp.sum(e, axis=-1, keepdims=True))

        def values(hd):
            outs[hd] = _dp(prob.pop(hd), qkv.pop(hd)[:, 2 * E:])

        lo = [_d0(hin[:, :D // 2], pltpu.bitcast(wqkv_v[hd, pl.ds(0, D // 4), :], BF16))
              for hd in range(KSPLIT)]
        for hd in range(KSPLIT):
            qkv[hd] = _d0(
                hin[:, D // 2:], pltpu.bitcast(wqkv_v[hd, pl.ds(D // 4, D // 4), :], BF16)) + lo[hd]
        ns = npv = 0
        first = []
        for it in range(KSPLIT, H + n_col):
            if it < H:
                qkv[it] = _dq(hin, pltpu.bitcast(wqkv_v[it], BF16))
            else:
                if it == H:
                    o1 = jnp.concatenate([outs[hd] for hd in range(HSPLIT)], axis=-1)
                first.append(_d1(o1, pltpu.bitcast(wo_v[it - H, pl.ds(0, K1), :], BF16)))
            while ns < H and ns <= it - LAG_S:
                scores(ns)
                ns += 1
            while npv < H and npv <= it - LAG_P:
                values(npv)
                npv += 1
        o2 = jnp.concatenate([outs[hd] for hd in range(HSPLIT, H)], axis=-1)
        o = jnp.concatenate(
            [_d2(o2, pltpu.bitcast(wo_v[j, pl.ds(K1, H * E // 2 - K1), :], BF16)) + first[j]
             for j in range(n_col)], axis=-1)
        res = x_v[rows, :].astype(F32) + o[M:] * g_v[rows, :]
        out_v[rows, :] = res.astype(out_v.dtype)
        return o[:M]

    def steps(i, mem):
        for u in range(UNROLL):
            mem = step(i * UNROLL + u, mem)
        rows = pl.ds(pl.multiple_of(i * UNROLL * seg, UNROLL * seg), UNROLL * seg)
        pltpu.make_async_copy(out_v.at[rows], out_hbm.at[rows], out_sem).start()
        return mem

    with jax.named_scope('p_scan'):
        jax.lax.fori_loop(0, S // seg // UNROLL, steps, mem_ref[...].astype(F32))
    pltpu.make_async_copy(out_v, out_hbm, out_sem).wait()


@functools.partial(jax.jit, static_argnames=("A_seg_len",))
def pallas_recurrent_scan__memory_aug_recurrent_mem_tr__mixer_s_mlp__prompt_kernel(
    A_x: jax.Array,
    A_mem0: jax.Array,
    A_Wq: jax.Array,
    A_Wk: jax.Array,
    A_Wv: jax.Array,
    A_Wo: jax.Array,
    A_seg_len: int,
    B_x: jax.Array,
    B_w1: jax.Array,
    B_w2: jax.Array,
    B_w3: jax.Array,
    B_w4: jax.Array,
):
    del B_x
    B, S, D = A_x.shape
    _, H, E = A_Wq.shape
    M = A_mem0.shape[1]
    F = B_w3.shape[1]
    seg = int(A_seg_len)
    assert B == 1 and S % ROWS == 0 and S % seg == 0 and E == LANES

    hbm = pl.BlockSpec(memory_space=pl.ANY)
    out = pl.pallas_call(
        functools.partial(_kernel, seg=seg),
        out_shape=jax.ShapeDtypeStruct((S, D), A_x.dtype),
        in_specs=[hbm, pl.BlockSpec(memory_space=pltpu.VMEM)] + [hbm] * 8,
        out_specs=hbm,
        scratch_shapes=[
            pltpu.VMEM((S, D), BF16),
            pltpu.VMEM((S, D), F32),
            pltpu.VMEM((2, ROWS1, D), BF16),
            pltpu.VMEM((S + 2 * HALO, D), F32),
            pltpu.VMEM((S, D), F32),
            pltpu.VMEM((S, D), A_x.dtype),
            pltpu.VMEM((D, D), BF16),
            pltpu.VMEM((D, D), BF16),
            pltpu.VMEM((D, F), BF16),
            pltpu.VMEM((F, D), BF16),
            pltpu.VMEM((3, D * H // 2, E), U32),
            pltpu.VMEM((3, 4, 64 * H // 8, E), U32),
            pltpu.VMEM((H, D // 2, 3 * E), U32),
            pltpu.VMEM((D // LANES, H * E // 2, LANES), U32),
            pltpu.SemaphoreType.DMA((S // ROWS1,)),
            pltpu.SemaphoreType.DMA((7,)),
            pltpu.SemaphoreType.DMA((D // LANES,)),
            pltpu.SemaphoreType.DMA(()),
        ],
        compiler_params=pltpu.CompilerParams(vmem_limit_bytes=120 * 1024 * 1024),
    )(
        A_x.reshape(S, D), A_mem0.reshape(M, D), A_Wq.reshape(D * H, E), A_Wk.reshape(D * H, E), A_Wv.reshape(D * H, E),
        A_Wo.reshape(H * E, D), B_w1, B_w2, B_w3, B_w4,
    )
    return out.reshape(B, S, D)
```

```python
import functools

import jax
import jax.numpy as jnp
import jax.experimental.pallas as pl
import jax.experimental.pallas.tpu as pltpu

F32 = jnp.float32
BF16 = jnp.bfloat16
U32 = jnp.uint32

LANES = 128
HALO = 8
ROWS = 256
FC = 512
UNROLL = 2
HSPLIT = 24
KSPLIT = 2
LAG_S = 1
LAG_P = 3
HIDE = True
W34_AT = 3
WA_AT = 2

_NN = (((1,), (0,)), ((), ()))
_NT = (((1,), (1,)), ((), ()))


def _dot(a, b, dims=_NN):
    return jax.lax.dot_general(a, b, dims, preferred_element_type=F32)


def _layernorm(x, eps=1e-5):
    d = x - jnp.mean(x, axis=-1, keepdims=True)
    return d * jax.lax.rsqrt(jnp.mean(d * d, axis=-1, keepdims=True) + eps)


def _recip(x):
    r = pl.reciprocal(x, approx=True)
    return r * (2.0 - x * r)


def _gelu(x):
    return jax.nn.gelu(x, approximate=True)


def _kernel(
    x_hbm, mem_ref, wq_hbm, wk_hbm, wv_hbm, wo_hbm, w1_hbm, w2_hbm, w3_hbm, w4_hbm,
    out_hbm,
    x_v, xn_v, h_v, g_v, out_v, w1_v, w2_v, w3_v, w4_v, stage_v, tmp_v, wo_v,
    x_sems, w_sems, qkv_sems, wo_sems, out_sem, *wqkv_v, seg,
):
    S, D = x_v.shape
    H, E = len(wqkv_v), LANES
    F = w3_v.shape[1]
    M = mem_ref.shape[0]
    L = M + seg
    n_col = D // LANES
    n_blk = S // ROWS
    DC = D // n_blk

    def block(i):
        start = i * ROWS
        return pl.ds(start if isinstance(i, int) else pl.multiple_of(start, ROWS), ROWS)

    def x_copy(i):
        return pltpu.make_async_copy(x_hbm.at[block(i)], x_v.at[block(i)], x_sems.at[i])

    w_copies = [
        pltpu.make_async_copy(src, dst, w_sems.at[i])
        for i, (src, dst) in enumerate(
            ((w1_hbm, w1_v), (w2_hbm, w2_v), (w3_hbm, w3_v), (w4_hbm, w4_v)))
    ]
    stage_bf = stage_v.bitcast(BF16)

    def qkv_copy(t, c):
        rows = pl.ds(pl.multiple_of(c * (DC * H), DC * H), DC * H)
        return pltpu.make_async_copy(
            (wq_hbm, wk_hbm, wv_hbm)[t].at[rows], stage_bf.at[t, rows],
            qkv_sems.at[t * n_blk + c])

    wo_bf = wo_v.bitcast(BF16)
    wo_copies = [
        pltpu.make_async_copy(
            wo_hbm.at[:, pl.ds(j * LANES, LANES)], wo_bf.at[j], wo_sems.at[j])
        for j in range(n_col)
    ]
    x_copy(0).start()
    w_copies[0].start()
    x_copy(1).start()

    h_v[pl.ds(0, HALO), :] = jnp.zeros((HALO, D), F32)
    h_v[pl.ds(HALO + S, HALO), :] = jnp.zeros((HALO, D), F32)
    g_v[block(0), :] = jnp.zeros((ROWS, D), F32)
    ln_v = out_v

    def norm_in(i):
        xn = _layernorm(x_v[block(i), :].astype(F32))
        xn_v[block(i), :] = xn
        ln_v[block(i), :] = _layernorm(xn).astype(BF16)

    def project(i):
        r0 = pl.multiple_of(i * ROWS, ROWS)
        h_v[pl.ds(r0 + HALO, ROWS), :] = _gelu(_dot(ln_v[block(i), :], w1_v[...]))

    with jax.named_scope('p_wait1'):
        x_copy(0).wait()
        norm_in(0)
        w_copies[0].wait()
    for i in range(2, n_blk):
        x_copy(i).start()
    w_copies[1].start()

    def stage1(i, carry):
        @pl.when(i == W34_AT)
        def _():
            w_copies[2].start()
            w_copies[3].start()

        @pl.when(i + 1 < n_blk)
        def _():
            x_copy(i + 1).wait()

        project(i)
        norm_in(jnp.minimum(i + 1, n_blk - 1))
        return carry

    with jax.named_scope('p_stage1'):
        jax.lax.fori_loop(0, n_blk, stage1, 0)

    with jax.named_scope('p_wait2'):
        w_copies[1].wait()
    C = D // 4

    def mix(i):
        r0 = pl.multiple_of(i * ROWS, ROWS)
        parts = []
        for c, shift in enumerate((-1, 1, -2, 2)):
            win = h_v[pl.ds(r0, ROWS + 2 * HALO), pl.ds(c * C, C)]
            parts.append(win[HALO + shift:HALO + shift + ROWS].astype(BF16))
        hs = _dot(jnp.concatenate(parts, axis=-1), w2_v[...])
        g_v[block(i), :] = hs + xn_v[block(i), :]

    def norm_mid(i):
        ln_v[block(i), :] = _layernorm(g_v[block(i), :]).astype(BF16)

    def stage2(i, carry):
        @pl.when(i == WA_AT)
        def _():
            for c in range(n_blk):
                for t in range(3):
                    qkv_copy(t, c).start()
            for c in wo_copies:
                c.start()

        norm_mid(jnp.maximum(i - 1, 0))
        mix(i)
        return carry

    with jax.named_scope('p_stage2'):
        jax.lax.fori_loop(0, n_blk, stage2, 0)
        norm_mid(n_blk - 1)

    with jax.named_scope('p_wait34'):
        w_copies[2].wait()
        w_copies[3].wait()

    def relayout(t, c):
        G = H // 8
        base = pl.multiple_of(c * (DC * H // 2), DC * H // 2)
        dst = pl.ds(pl.multiple_of(c * (DC // 2), DC // 2), DC // 2)
        for j0 in range(4):
            tmp_v[t, j0] = stage_v[t, pl.ds(base + j0, DC * G, stride=4), :]
        for j0 in range(4):
            for j1 in range(G):
                w = tmp_v[t, j0, pl.ds(j1, DC, stride=G), :]
                for half, bits in enumerate((w, w >> 16)):
                    wqkv_v[2 * (4 * j1 + j0) + half][dst, pl.ds(t * E, E)] = pltpu.bitcast(
                        bits.astype(jnp.uint16), U32)

    def stage3(i, carry):
        if HIDE:
            for t in range(3):
                qkv_copy(t, i).wait()
        ln = ln_v[block(i), :]
        acc = g_v[block(i), :]
        for f in range(F // FC):
            u = _gelu(_dot(ln, w3_v[:, pl.ds(f * FC, FC)])).astype(BF16)
            acc = _dot(u, w4_v[pl.ds(f * FC, FC), :]) + acc
            if HIDE and f % 2 == 1:
                relayout(f // 2, i)
        g_v[block(i), :] = jax.nn.silu(acc)
        return carry

    with jax.named_scope('p_stage3'):
        jax.lax.fori_loop(0, n_blk, stage3, 0)
    if not HIDE:
        def relayout_all(c, carry):
            for t in range(3):
                qkv_copy(t, c).wait()
            for t in range(3):
                relayout(t, c)
            return carry
        with jax.named_scope('p_relayout'):
            jax.lax.fori_loop(0, n_blk, relayout_all, 0)
    with jax.named_scope('p_waitA'):
        for c in wo_copies:
            c.wait()

    scale = E ** -0.5
    qi = jax.lax.broadcasted_iota(jnp.int32, (L, L), 0)
    ki = jax.lax.broadcasted_iota(jnp.int32, (L, L), 1)
    mask = (qi < M) | (qi >= ki)
    K1 = HSPLIT * E // 2

    def step(s, mem):
        rows = pl.ds(pl.multiple_of(s * seg, seg), seg)
        hin = jnp.concatenate([mem, xn_v[rows, :]], axis=0)
        qkv, prob, outs = {}, {}, {}

        def scores(hd):
            sc = _dot(qkv[hd][:, :E], qkv[hd][:, E:2 * E], _NT) * scale
            sc = jnp.where(mask, sc, -1e9)
            e = jnp.exp(sc - jnp.max(sc, axis=-1, keepdims=True))
            prob[hd] = e * _recip(jnp.sum(e, axis=-1, keepdims=True))

        def values(hd):
            outs[hd] = _dot(prob.pop(hd), qkv.pop(hd)[:, 2 * E:])

        lo = [_dot(hin[:, :D // 2], pltpu.bitcast(wqkv_v[hd][pl.ds(0, D // 4), :], BF16))
              for hd in range(KSPLIT)]
        ns = npv = 0
        first = []
        for it in range(H + n_col):
            if it < KSPLIT:
                qkv[it] = _dot(hin[:, D // 2:], pltpu.bitcast(
                    wqkv_v[it][pl.ds(D // 4, D // 4), :], BF16)) + lo[it]
            elif it < H:
                qkv[it] = _dot(hin, pltpu.bitcast(wqkv_v[it][...], BF16))
            else:
                if it == H:
                    o1 = jnp.concatenate([outs[hd] for hd in range(HSPLIT)], axis=-1)
                first.append(_dot(o1, pltpu.bitcast(wo_v[it - H, pl.ds(0, K1), :], BF16)))
            while ns < H and ns <= it - LAG_S:
                scores(ns)
                ns += 1
            while npv < H and npv <= it - LAG_P:
                values(npv)
                npv += 1
        o2 = jnp.concatenate([outs[hd] for hd in range(HSPLIT, H)], axis=-1)
        o = jnp.concatenate(
            [_dot(o2, pltpu.bitcast(wo_v[j, pl.ds(K1, H * E // 2 - K1), :], BF16)) + first[j]
             for j in range(n_col)], axis=-1)
        res = x_v[rows, :].astype(F32) + o[M:] * g_v[rows, :]
        out_v[rows, :] = res.astype(out_v.dtype)
        return o[:M]

    def steps(i, mem):
        for u in range(UNROLL):
            mem = step(i * UNROLL + u, mem)
        rows = pl.ds(pl.multiple_of(i * UNROLL * seg, UNROLL * seg), UNROLL * seg)
        pltpu.make_async_copy(out_v.at[rows], out_hbm.at[rows], out_sem).start()
        return mem

    with jax.named_scope('p_scan'):
        jax.lax.fori_loop(0, S // seg // UNROLL, steps, mem_ref[...].astype(F32))
    pltpu.make_async_copy(out_v, out_hbm, out_sem).wait()


@functools.partial(jax.jit, static_argnames=("A_seg_len",))
def pallas_recurrent_scan__memory_aug_recurrent_mem_tr__mixer_s_mlp__prompt_kernel(
    A_x: jax.Array,
    A_mem0: jax.Array,
    A_Wq: jax.Array,
    A_Wk: jax.Array,
    A_Wv: jax.Array,
    A_Wo: jax.Array,
    A_seg_len: int,
    B_x: jax.Array,
    B_w1: jax.Array,
    B_w2: jax.Array,
    B_w3: jax.Array,
    B_w4: jax.Array,
):
    del B_x
    B, S, D = A_x.shape
    _, H, E = A_Wq.shape
    M = A_mem0.shape[1]
    F = B_w3.shape[1]
    seg = int(A_seg_len)
    assert B == 1 and S % ROWS == 0 and S % seg == 0 and E == LANES
    n_blk = S // ROWS

    hbm = pl.BlockSpec(memory_space=pl.ANY)
    out = pl.pallas_call(
        functools.partial(_kernel, seg=seg),
        out_shape=jax.ShapeDtypeStruct((S, D), A_x.dtype),
        in_specs=[hbm, pl.BlockSpec(memory_space=pltpu.VMEM)] + [hbm] * 8,
        out_specs=hbm,
        scratch_shapes=[
            pltpu.VMEM((S, D), BF16),
            pltpu.VMEM((S, D), F32),
            pltpu.VMEM((S + 2 * HALO, D), F32),
            pltpu.VMEM((S, D), F32),
            pltpu.VMEM((S, D), BF16),
            pltpu.VMEM((D, D), BF16),
            pltpu.VMEM((D, D), BF16),
            pltpu.VMEM((D, F), BF16),
            pltpu.VMEM((F, D), BF16),
            pltpu.VMEM((3, D * H // 2, E), U32),
            pltpu.VMEM((3, 4, D // n_blk * H // 8, E), U32),
            pltpu.VMEM((D // LANES, H * E // 2, LANES), U32),
            pltpu.SemaphoreType.DMA((n_blk,)),
            pltpu.SemaphoreType.DMA((4,)),
            pltpu.SemaphoreType.DMA((3 * n_blk,)),
            pltpu.SemaphoreType.DMA((D // LANES,)),
            pltpu.SemaphoreType.DMA(()),
        ] + [pltpu.VMEM((D // 2, 3 * E), U32)] * H,
        compiler_params=pltpu.CompilerParams(vmem_limit_bytes=124 * 1024 * 1024),
    )(
        A_x.reshape(S, D), A_mem0.reshape(M, D),
        A_Wq.reshape(D * H, E), A_Wk.reshape(D * H, E), A_Wv.reshape(D * H, E),
        A_Wo.reshape(H * E, D), B_w1, B_w2, B_w3, B_w4,
    )
    return out.reshape(B, S, D)
```

```python
import functools

import jax
import jax.numpy as jnp
import jax.experimental.pallas as pl
import jax.experimental.pallas.tpu as pltpu

F32 = jnp.float32
BF16 = jnp.bfloat16
U32 = jnp.uint32

LANES = 128
HALO = 8
ROWS = 256
FC = 512
UNROLL = 2
HSPLIT = 24
KSPLIT = 2
LAG_S = 1
LAG_P = 3
HIDE = True
RES_AT = 3
MODE = 0
W34_AT = 3
WA_AT = 2

_NN = (((1,), (0,)), ((), ()))
_NT = (((1,), (1,)), ((), ()))


def _dot(a, b, dims=_NN):
    return jax.lax.dot_general(a, b, dims, preferred_element_type=F32)


def _layernorm(x, eps=1e-5):
    d = x - jnp.mean(x, axis=-1, keepdims=True)
    return d * jax.lax.rsqrt(jnp.mean(d * d, axis=-1, keepdims=True) + eps)


def _recip(x):
    r = pl.reciprocal(x, approx=True)
    return r * (2.0 - x * r)


def _gelu(x):
    return jax.nn.gelu(x, approximate=True)


def _kernel(
    x_hbm, mem_ref, wq_hbm, wk_hbm, wv_hbm, wo_hbm, w1_hbm, w2_hbm, w3_hbm, w4_hbm,
    out_hbm,
    x_v, xn_v, h_v, lhs_v, g_v, out_v, w1_v, w2_v, w3_v, w4_v, stage_v, tmp_v, wo_v,
    x_sems, w_sems, qkv_sems, out_sem, *wqkv_v, seg,
):
    S, D = x_v.shape
    H, E = len(wqkv_v), LANES
    F = w3_hbm.shape[1]
    M = mem_ref.shape[0]
    L = M + seg
    n_col = D // LANES
    n_blk = S // ROWS
    DC = D // n_blk

    def block(i):
        start = i * ROWS
        return pl.ds(start if isinstance(i, int) else pl.multiple_of(start, ROWS), ROWS)

    def x_copy(i):
        return pltpu.make_async_copy(x_hbm.at[block(i)], x_v.at[block(i)], x_sems.at[i])

    def weight_copies(t):
        src = (w1_hbm, w2_hbm, w3_hbm, w4_hbm, wo_hbm)[t]
        dst = (w1_v, w2_v, w3_v, w4_v, wo_v)[t].bitcast(BF16)
        return [
            pltpu.make_async_copy(
                src.at[:, pl.ds(j * LANES, LANES)], dst.at[j], w_sems.at[t])
            for j in range(dst.shape[0])
        ]

    def start_weight(t):
        for c in weight_copies(t):
            c.start()

    def wait_weight(t):
        for c in weight_copies(t):
            c.wait()

    def weight(ref, k0, k, n0, n):
        tiles = [ref[j, pl.ds(k0 // 2, k // 2), :]
                 for j in range(n0 // LANES, (n0 + n) // LANES)]
        return pltpu.bitcast(jnp.concatenate(tiles, axis=-1), BF16)

    stage_bf = stage_v.bitcast(BF16)

    def qkv_copy(t, c):
        rows = pl.ds(pl.multiple_of(c * (DC * H), DC * H), DC * H)
        return pltpu.make_async_copy(
            (wq_hbm, wk_hbm, wv_hbm)[t].at[rows], stage_bf.at[t, rows],
            qkv_sems.at[t * n_blk + c])

    x_copy(0).start()
    start_weight(0)
    x_copy(1).start()

    HALF = ROWS // 2

    def half(i, p, offset=0, extra=0):
        start = i * ROWS + p * HALF
        if not isinstance(start, int):
            start = pl.multiple_of(start, HALF)
        return pl.ds(start + offset, HALF + extra)

    def following(i):
        return jnp.minimum(i + 1, n_blk - 1)

    def put_lhs(value):
        lhs_v[...] = pltpu.bitcast(value, U32)

    def get_lhs():
        return pltpu.bitcast(lhs_v[...], BF16)

    h_v[pl.ds(0, HALO), :] = jnp.zeros((HALO, D), F32)
    h_v[pl.ds(HALO + S, HALO), :] = jnp.zeros((HALO, D), F32)

    def norm_in(rows):
        xn = _layernorm(x_v[rows, :].astype(F32))
        return xn, _layernorm(xn).astype(BF16)

    with jax.named_scope('p_wait1'):
        x_copy(0).wait()
        xn_v[half(0, 0), :], ln = norm_in(half(0, 0))
        put_lhs(ln)
        wait_weight(0)
    for i in range(2, n_blk):
        x_copy(i).start()
    start_weight(1)

    def stage1(i, carry):
        @pl.when(i == W34_AT)
        def _():
            start_weight(2)
            start_weight(3)

        @pl.when(i + 1 < n_blk)
        def _():
            x_copy(i + 1).wait()

        ln0 = get_lhs()
        xn1, ln1 = norm_in(half(i, 1))
        xn2, ln2 = norm_in(half(following(i), 0))
        h0 = _gelu(_dot(ln0, weight(w1_v, 0, D, 0, D)))
        h1 = _gelu(_dot(ln1, weight(w1_v, 0, D, 0, D)))
        xn_v[half(i, 1), :] = xn1
        xn_v[half(following(i), 0), :] = xn2
        put_lhs(ln2)
        h_v[half(i, 0, HALO), :] = h0
        h_v[half(i, 1, HALO), :] = h1
        return carry

    with jax.named_scope('p_stage1'):
        jax.lax.fori_loop(0, n_blk, stage1, 0)

    C = D // 4

    def shifted(i, p):
        parts = []
        for c, shift in enumerate((-1, 1, -2, 2)):
            win = h_v[half(i, p, 0, 2 * HALO), pl.ds(c * C, C)]
            parts.append(win[HALO + shift:HALO + shift + HALF].astype(BF16))
        return jnp.concatenate(parts, axis=-1)

    def stage2(i, carry):
        @pl.when(i == WA_AT)
        def _():
            for c in range(n_blk):
                for t in range(3):
                    qkv_copy(t, c).start()
            start_weight(4)

        hs0 = get_lhs()
        hs1 = shifted(i, 1)
        hs2 = shifted(following(i), 0)
        y0 = _dot(hs0, weight(w2_v, 0, D, 0, D)) + xn_v[half(i, 0), :]
        y1 = _dot(hs1, weight(w2_v, 0, D, 0, D)) + xn_v[half(i, 1), :]
        put_lhs(hs2)
        g_v[half(i, 0), :] = y0
        g_v[half(i, 1), :] = y1
        return carry

    with jax.named_scope('p_stage2'):
        put_lhs(shifted(0, 0))
        wait_weight(1)
        jax.lax.fori_loop(0, n_blk, stage2, 0)

    def relayout(t, c):
        G = H // 8
        base = pl.multiple_of(c * (DC * H // 2), DC * H // 2)
        dst = pl.ds(pl.multiple_of(c * (DC // 2), DC // 2), DC // 2)
        for j0 in range(4):
            tmp_v[t, j0] = stage_v[t, pl.ds(base + j0, DC * G, stride=4), :]
        for j0 in range(4):
            for j1 in range(G):
                w = tmp_v[t, j0, pl.ds(j1, DC, stride=G), :]
                for odd, bits in enumerate((w, w >> 16)):
                    wqkv_v[2 * (4 * j1 + j0) + odd][dst, pl.ds(t * E, E)] = pltpu.bitcast(
                        bits.astype(jnp.uint16), U32)

    def norm_mid(rows):
        return _layernorm(g_v[rows, :]).astype(BF16)

    def stage3(i, carry):
        for t in range(3):
            qkv_copy(t, i).wait()
        ln0, ln1 = get_lhs(), norm_mid(half(i, 1))
        ln = jnp.concatenate([ln0, ln1], axis=0)
        acc = g_v[block(i), :]
        ln2 = norm_mid(half(following(i), 0))
        for f in range(F // FC):
            w = weight(w3_v, 0, D, f * FC, FC)
            if f == 0:
                u = jnp.concatenate([_dot(ln0, w), _dot(ln1, w)], axis=0)
            else:
                u = _dot(ln, w)
            acc = _dot(_gelu(u).astype(BF16), weight(w4_v, f * FC, FC, 0, D)) + acc
            if MODE == 0 and f % 2 == 1:
                relayout(f // 2, i)
        if MODE == 2:
            for t in range(3):
                relayout(t, i)
        put_lhs(ln2)
        g_v[block(i), :] = acc * _recip(1.0 + jnp.exp(-acc))
        return carry

    with jax.named_scope('p_stage3'):
        put_lhs(norm_mid(half(0, 0)))
        wait_weight(2)
        wait_weight(3)
        jax.lax.fori_loop(0, n_blk, stage3, 0)
    with jax.named_scope('p_waitA'):
        wait_weight(4)

    scale = E ** -0.5
    qi = jax.lax.broadcasted_iota(jnp.int32, (L, L), 0)
    ki = jax.lax.broadcasted_iota(jnp.int32, (L, L), 1)
    mask = (qi < M) | (qi >= ki)
    K1 = HSPLIT * E // 2

    def step(s, mem):
        rows = pl.ds(pl.multiple_of(s * seg, seg), seg)
        hin = jnp.concatenate([mem, xn_v[rows, :]], axis=0)
        qkv, prob, outs = {}, {}, {}

        def scores(hd):
            sc = _dot(qkv[hd][:, :E], qkv[hd][:, E:2 * E], _NT) * scale
            sc = jnp.where(mask, sc, -1e9)
            e = jnp.exp(sc - jnp.max(sc, axis=-1, keepdims=True))
            prob[hd] = e * _recip(jnp.sum(e, axis=-1, keepdims=True))

        def values(hd):
            outs[hd] = _dot(prob.pop(hd), qkv.pop(hd)[:, 2 * E:])

        lo = [_dot(hin[:, :D // 2], pltpu.bitcast(wqkv_v[hd][pl.ds(0, D // 4), :], BF16))
              for hd in range(KSPLIT)]
        ns = npv = 0
        first = []
        for it in range(H + n_col):
            if it < KSPLIT:
                qkv[it] = _dot(hin[:, D // 2:], pltpu.bitcast(
                    wqkv_v[it][pl.ds(D // 4, D // 4), :], BF16)) + lo[it]
            elif it < H:
                qkv[it] = _dot(hin, pltpu.bitcast(wqkv_v[it][...], BF16))
            else:
                if it == H:
                    o1 = jnp.concatenate([outs[hd] for hd in range(HSPLIT)], axis=-1)
                first.append(_dot(o1, pltpu.bitcast(wo_v[it - H, pl.ds(0, K1), :], BF16)))
            while ns < H and ns <= it - LAG_S:
                scores(ns)
                ns += 1
            while npv < H and npv <= it - LAG_P:
                values(npv)
                npv += 1
        o2 = jnp.concatenate([outs[hd] for hd in range(HSPLIT, H)], axis=-1)
        o = jnp.concatenate(
            [_dot(o2, pltpu.bitcast(wo_v[j, pl.ds(K1, H * E // 2 - K1), :], BF16)) + first[j]
             for j in range(n_col)], axis=-1)
        res = x_v[rows, :].astype(F32) + o[M:] * g_v[rows, :]
        out_v[rows, :] = res.astype(out_v.dtype)
        return o[:M]

    def steps(i, mem):
        for u in range(UNROLL):
            mem = step(i * UNROLL + u, mem)
        rows = pl.ds(pl.multiple_of(i * UNROLL * seg, UNROLL * seg), UNROLL * seg)
        pltpu.make_async_copy(out_v.at[rows], out_hbm.at[rows], out_sem).start()
        return mem

    with jax.named_scope('p_scan'):
        jax.lax.fori_loop(0, S // seg // UNROLL, steps, mem_ref[...].astype(F32))
    pltpu.make_async_copy(out_v, out_hbm, out_sem).wait()


@functools.partial(jax.jit, static_argnames=("A_seg_len",))
def pallas_recurrent_scan__memory_aug_recurrent_mem_tr__mixer_s_mlp__prompt_kernel(
    A_x: jax.Array,
    A_mem0: jax.Array,
    A_Wq: jax.Array,
    A_Wk: jax.Array,
    A_Wv: jax.Array,
    A_Wo: jax.Array,
    A_seg_len: int,
    B_x: jax.Array,
    B_w1: jax.Array,
    B_w2: jax.Array,
    B_w3: jax.Array,
    B_w4: jax.Array,
):
    del B_x
    B, S, D = A_x.shape
    _, H, E = A_Wq.shape
    M = A_mem0.shape[1]
    F = B_w3.shape[1]
    seg = int(A_seg_len)
    assert B == 1 and S % ROWS == 0 and S % seg == 0 and E == LANES
    n_blk = S // ROWS

    def by_column_tile(k, n):
        return pltpu.VMEM((n // LANES, k // 2, LANES), U32)

    hbm = pl.BlockSpec(memory_space=pl.ANY)
    out = pl.pallas_call(
        functools.partial(_kernel, seg=seg),
        out_shape=jax.ShapeDtypeStruct((S, D), A_x.dtype),
        in_specs=[hbm, pl.BlockSpec(memory_space=pltpu.VMEM)] + [hbm] * 8,
        out_specs=hbm,
        scratch_shapes=[
            pltpu.VMEM((S, D), BF16),
            pltpu.VMEM((S, D), F32),
            pltpu.VMEM((S + 2 * HALO, D), F32),
            pltpu.VMEM((ROWS // 4, D), U32),
            pltpu.VMEM((S, D), F32),
            pltpu.VMEM((S, D), BF16),
            by_column_tile(D, D),
            by_column_tile(D, D),
            by_column_tile(D, F),
            by_column_tile(F, D),
            pltpu.VMEM((3, D * H // 2, E), U32),
            pltpu.VMEM((3, 4, D // n_blk * H // 8, E), U32),
            by_column_tile(H * E, D),
            pltpu.SemaphoreType.DMA((n_blk,)),
            pltpu.SemaphoreType.DMA((5,)),
            pltpu.SemaphoreType.DMA((3 * n_blk,)),
            pltpu.SemaphoreType.DMA(()),
        ] + [pltpu.VMEM((D // 2, 3 * E), U32)] * H,
        compiler_params=pltpu.CompilerParams(vmem_limit_bytes=124 * 1024 * 1024),
    )(
        A_x.reshape(S, D), A_mem0.reshape(M, D),
        A_Wq.reshape(D * H, E), A_Wk.reshape(D * H, E), A_Wv.reshape(D * H, E),
        A_Wo.reshape(H * E, D), B_w1, B_w2, B_w3, B_w4,
    )
    return out.reshape(B, S, D)
```

```python
import functools

import jax
import jax.numpy as jnp
import jax.experimental.pallas as pl
import jax.experimental.pallas.tpu as pltpu

F32 = jnp.float32
BF16 = jnp.bfloat16
U32 = jnp.uint32

LANES = 128
SUBLANES = 8
HALO = SUBLANES
ROWS = 256
HALF = ROWS // 2
FC = 512
WAIT_AT = 3
UNROLL = 2
KSPLIT = 2
LAG_SCORES = 1
LAG_VALUES = 3
LATE_HEADS = 8

_NN = (((1,), (0,)), ((), ()))
_NT = (((1,), (1,)), ((), ()))


def _dot(a, b, dims=_NN):
    return jax.lax.dot_general(a, b, dims, preferred_element_type=F32)


def _layernorm(x, eps=1e-5):
    d = x - jnp.mean(x, axis=-1, keepdims=True)
    return d * jax.lax.rsqrt(jnp.mean(d * d, axis=-1, keepdims=True) + eps)


def _gelu(x):
    return jax.nn.gelu(x, approximate=True)


def _softmax(x):
    e = jnp.exp(x - jnp.max(x, axis=-1, keepdims=True))
    total = jnp.sum(e, axis=-1, keepdims=True)
    r = pl.reciprocal(total, approx=True)
    return e * (r * (2.0 - total * r))


def _kernel(
    x_hbm, mem_ref, wq_hbm, wk_hbm, wv_hbm, wo_hbm, w1_hbm, w2_hbm, w3_hbm, w4_hbm,
    out_hbm,
    x_v, xn_v, h_v, lhs_v, gate_v, out_v, w1_v, w2_v, w3_v, w4_v, wo_v, stored_v, tmp_v,
    x_sems, w_sems, qkv_sems, out_sem, *wqkv_v, seg,
):
    S, D = x_v.shape
    H, E = len(wqkv_v), LANES
    F = w3_hbm.shape[1]
    M = mem_ref.shape[0]
    n_blk = S // ROWS
    n_col = D // LANES
    DC = D // n_blk

    def aligned_rows(start, align, size, offset=0):
        if not isinstance(start, int):
            start = pl.multiple_of(start, align)
        return pl.ds(start + offset, size)

    def block(i):
        return aligned_rows(i * ROWS, ROWS, ROWS)

    def half(i, p, offset=0, extra=0):
        return aligned_rows(i * ROWS + p * HALF, HALF, HALF + extra, offset)

    def following(i):
        return jnp.minimum(i + 1, n_blk - 1)

    def x_copy(i):
        return pltpu.make_async_copy(x_hbm.at[block(i)], x_v.at[block(i)], x_sems.at[i])

    def qkv_copy(t, c):
        return pltpu.make_async_copy(
            (wq_hbm, wk_hbm, wv_hbm)[t].at[aligned_rows(c * (DC * H), DC * H, DC * H)],
            stored_v.bitcast(BF16).at[t, c, pl.ds(0, DC * H)],
            qkv_sems.at[t * n_blk + c])

    F1 = (WAIT_AT + 1) * FC
    pieces = dict(
        w1=(w1_hbm, w1_v, 0, D, 0, D),
        w2=(w2_hbm, w2_v, 0, D, 0, D),
        w3_early=(w3_hbm, w3_v, 0, D, 0, F1),
        w4_early=(w4_hbm, w4_v, 0, F1, 0, D),
        w3_late=(w3_hbm, w3_v, 0, D, F1, F - F1),
        w4_late=(w4_hbm, w4_v, F1, F - F1, 0, D),
        wo=(wo_hbm, wo_v, 0, H * E, 0, D),
    )

    def weight_copies(names):
        copies = []
        for name in names:
            src, dst, k0, k, n0, n = pieces[name]
            copies += [
                pltpu.make_async_copy(
                    src.at[pl.ds(k0, k), pl.ds(j * LANES, LANES)],
                    dst.bitcast(BF16).at[j, pl.ds(k0, k)],
                    w_sems.at[list(pieces).index(name)])
                for j in range(n0 // LANES, (n0 + n) // LANES)
            ]
        return copies

    def start_weights(*names):
        for c in weight_copies(names):
            c.start()

    def wait_weights(*names):
        for c in weight_copies(names):
            c.wait()

    def weight(ref, k0, k, n0, n):
        tiles = [ref[j, pl.ds(k0 // 2, k // 2), :]
                 for j in range(n0 // LANES, (n0 + n) // LANES)]
        return pltpu.bitcast(jnp.concatenate(tiles, axis=-1), BF16)

    def put_lhs(value):
        lhs_v[...] = pltpu.bitcast(value, U32)

    def get_lhs():
        return pltpu.bitcast(lhs_v[...], BF16)

    x_copy(0).start()
    start_weights("w1")
    x_copy(1).start()

    h_v[pl.ds(0, HALO), :] = jnp.zeros((HALO, D), F32)
    h_v[pl.ds(HALO + S, HALO), :] = jnp.zeros((HALO, D), F32)

    def normalise(rows):
        xn = _layernorm(x_v[rows, :].astype(F32))
        return xn, _layernorm(xn).astype(BF16)

    def stage1(i, carry):
        @pl.when(i == 1)
        def _():
            start_weights("w3_early", "w4_early")

        @pl.when(i + 1 < n_blk)
        def _():
            x_copy(i + 1).wait()

        ln0 = get_lhs()
        xn1, ln1 = normalise(half(i, 1))
        xn2, ln2 = normalise(half(following(i), 0))
        h0 = _gelu(_dot(ln0, weight(w1_v, 0, D, 0, D)))
        h1 = _gelu(_dot(ln1, weight(w1_v, 0, D, 0, D)))
        xn_v[half(i, 1), :] = xn1
        xn_v[half(following(i), 0), :] = xn2
        put_lhs(ln2)
        h_v[half(i, 0, HALO), :] = h0
        h_v[half(i, 1, HALO), :] = h1
        return carry

    x_copy(0).wait()
    xn_v[half(0, 0), :], ln = normalise(half(0, 0))
    put_lhs(ln)
    wait_weights("w1")
    for i in range(2, n_blk):
        x_copy(i).start()
    start_weights("w2")
    jax.lax.fori_loop(0, n_blk, stage1, 0)

    def shifted(i, p):
        parts = []
        for c, shift in enumerate((-1, 1, -2, 2)):
            window = h_v[half(i, p, 0, 2 * HALO), pl.ds(c * D // 4, D // 4)]
            parts.append(window[HALO + shift:HALO + shift + HALF].astype(BF16))
        return jnp.concatenate(parts, axis=-1)

    def relayout(t, c):
        G = H // SUBLANES
        dst = aligned_rows(c * (DC // 2), DC // 2, DC // 2)
        for j0 in range(4):
            tmp_v[t, j0, pl.ds(0, DC * G), :] = stored_v[t, c, pl.ds(j0, DC * G, stride=4), :]
        for j0 in range(4):
            for j1 in range(G):
                w = tmp_v[t, j0, pl.ds(j1, DC, stride=G), :]
                for odd, bits in enumerate((w, w >> 16)):
                    wqkv_v[2 * (4 * j1 + j0) + odd][dst, pl.ds(t * E, E)] = pltpu.bitcast(
                        bits.astype(jnp.uint16), U32)

    def start_qkv(c):
        for t in range(3):
            qkv_copy(t, c).start()

    def stage2(i, carry):
        @pl.when(i + 1 < n_blk)
        def _():
            start_qkv(i + 1)

        @pl.when(i == 2)
        def _():
            start_weights("wo")

        hs0, hs1 = get_lhs(), shifted(i, 1)
        hs2 = shifted(following(i), 0)
        y0 = _dot(hs0, weight(w2_v, 0, D, 0, D)) + xn_v[half(i, 0), :]
        y1 = _dot(hs1, weight(w2_v, 0, D, 0, D)) + xn_v[half(i, 1), :]
        ln0, ln1 = _layernorm(y0).astype(BF16), _layernorm(y1).astype(BF16)
        ln = jnp.concatenate([ln0, ln1], axis=0)
        acc = jnp.concatenate([y0, y1], axis=0)
        for f in range(F // FC):
            w3 = weight(w3_v, 0, D, f * FC, FC)
            if f == 0:
                u = jnp.concatenate([_dot(ln0, w3), _dot(ln1, w3)], axis=0)
            else:
                u = _dot(ln, w3)
            acc = _dot(_gelu(u).astype(BF16), weight(w4_v, f * FC, FC, 0, D)) + acc
            if f == WAIT_AT:
                @pl.when(i == 0)
                def _():
                    wait_weights("w3_late", "w4_late")

                for t in range(3):
                    qkv_copy(t, i).wait()
                for t in range(3):
                    relayout(t, i)
        put_lhs(hs2)
        gate_v[block(i), :] = jax.nn.silu(acc)
        return carry

    put_lhs(shifted(0, 0))
    wait_weights("w2", "w3_early", "w4_early")
    start_weights("w3_late", "w4_late")
    start_qkv(0)
    jax.lax.fori_loop(0, n_blk, stage2, 0)
    wait_weights("wo")

    L = M + seg
    query = jax.lax.broadcasted_iota(jnp.int32, (L, L), 0)
    key = jax.lax.broadcasted_iota(jnp.int32, (L, L), 1)
    mask = (query < M) | (query >= key)
    early = H - LATE_HEADS

    def step(s, mem):
        rows = aligned_rows(s * seg, seg, seg)
        tokens = jnp.concatenate([mem, xn_v[rows, :]], axis=0)

        def project(hd, k0, k):
            w = pltpu.bitcast(wqkv_v[hd][pl.ds(k0 // 2, k // 2), :], BF16)
            return _dot(tokens[:, k0:k0 + k], w)

        started = [project(hd, 0, D // 2) for hd in range(KSPLIT)]
        qkv, prob, heads, partial = [], [], [], []
        for it in range(H + n_col):
            if it < KSPLIT:
                qkv.append(project(it, D // 2, D // 2) + started[it])
            elif it < H:
                qkv.append(project(it, 0, D))
            else:
                if it == H:
                    o = jnp.concatenate(heads[:early], axis=-1)
                partial.append(_dot(o, weight(wo_v, 0, early * E, (it - H) * LANES, LANES)))
            if len(prob) < H and len(prob) <= it - LAG_SCORES:
                t = qkv[len(prob)]
                scores = _dot(t[:, :E], t[:, E:2 * E], _NT) * E ** -0.5
                prob.append(_softmax(jnp.where(mask, scores, -1e9)))
            if len(heads) < H and len(heads) <= it - LAG_VALUES:
                heads.append(_dot(prob[len(heads)], qkv[len(heads)][:, 2 * E:]))
        o = jnp.concatenate(heads[early:], axis=-1)
        o = jnp.concatenate(
            [_dot(o, weight(wo_v, early * E, LATE_HEADS * E, j * LANES, LANES)) + partial[j]
             for j in range(n_col)], axis=-1)
        out = x_v[rows, :].astype(F32) + o[M:] * gate_v[rows, :]
        out_v[rows, :] = out.astype(out_v.dtype)
        return o[:M]

    def steps(i, mem):
        for u in range(UNROLL):
            mem = step(i * UNROLL + u, mem)
        rows = aligned_rows(i * (UNROLL * seg), UNROLL * seg, UNROLL * seg)
        pltpu.make_async_copy(out_v.at[rows], out_hbm.at[rows], out_sem).start()
        return mem

    jax.lax.fori_loop(0, S // (UNROLL * seg), steps, mem_ref[...].astype(F32))
    pltpu.make_async_copy(out_v, out_hbm, out_sem).wait()


@functools.partial(jax.jit, static_argnames=("A_seg_len",))
def pallas_recurrent_scan__memory_aug_recurrent_mem_tr__mixer_s_mlp__prompt_kernel(
    A_x: jax.Array,
    A_mem0: jax.Array,
    A_Wq: jax.Array,
    A_Wk: jax.Array,
    A_Wv: jax.Array,
    A_Wo: jax.Array,
    A_seg_len: int,
    B_x: jax.Array,
    B_w1: jax.Array,
    B_w2: jax.Array,
    B_w3: jax.Array,
    B_w4: jax.Array,
):
    del B_x
    B, S, D = A_x.shape
    _, H, E = A_Wq.shape
    M = A_mem0.shape[1]
    F = B_w3.shape[1]
    seg = int(A_seg_len)
    n_blk = S // ROWS
    assert B == 1 and E == LANES and H % SUBLANES == 0 and M % SUBLANES == 0
    assert S % ROWS == 0 and S % (UNROLL * seg) == 0 and F % FC == 0

    def by_column_tile(k, n):
        return pltpu.VMEM((n // LANES, k // 2, LANES), U32)

    words = D // n_blk * H // 2
    hbm = pl.BlockSpec(memory_space=pl.ANY)
    out = pl.pallas_call(
        functools.partial(_kernel, seg=seg),
        out_shape=jax.ShapeDtypeStruct((S, D), A_x.dtype),
        in_specs=[hbm, pl.BlockSpec(memory_space=pltpu.VMEM)] + [hbm] * 8,
        out_specs=hbm,
        scratch_shapes=[
            pltpu.VMEM((S, D), A_x.dtype),
            pltpu.VMEM((S, D), F32),
            pltpu.VMEM((S + 2 * HALO, D), F32),
            pltpu.VMEM((HALF // 2, D), U32),
            pltpu.VMEM((S, D), F32),
            pltpu.VMEM((S, D), A_x.dtype),
            by_column_tile(D, D),
            by_column_tile(D, D),
            by_column_tile(D, F),
            by_column_tile(F, D),
            by_column_tile(H * E, D),
            pltpu.VMEM((3, n_blk, words + SUBLANES, E), U32),
            pltpu.VMEM((3, 4, words // 4 + SUBLANES, E), U32),
            pltpu.SemaphoreType.DMA((n_blk,)),
            pltpu.SemaphoreType.DMA((7,)),
            pltpu.SemaphoreType.DMA((3 * n_blk,)),
            pltpu.SemaphoreType.DMA(()),
        ] + [pltpu.VMEM((D // 2, 3 * E), U32)] * H,
        compiler_params=pltpu.CompilerParams(vmem_limit_bytes=124 * 1024 * 1024),
    )(
        A_x.reshape(S, D), A_mem0.reshape(M, D),
        A_Wq.reshape(D * H, E), A_Wk.reshape(D * H, E), A_Wv.reshape(D * H, E),
        A_Wo.reshape(H * E, D), B_w1, B_w2, B_w3, B_w4,
    )
    return out.reshape(B, S, D)
```

```python
import functools

import jax
import jax.numpy as jnp
import jax.experimental.pallas as pl
import jax.experimental.pallas.tpu as pltpu

F32 = jnp.float32
BF16 = jnp.bfloat16
U32 = jnp.uint32

LANES = 128
SUBLANES = 8
HALO = SUBLANES
ROWS = 256
HALF = ROWS // 2
FC = 512
WAIT_AT = 3
UNROLL = 2
FEW = SUBLANES
LAG_SCORES = 1
LAG_VALUES = 3
LAG_OUT = 12
TAIL = 4
OUT_HEADS = 2

MASKED = -1e9
LOG2E = 1.4426950408889634

_NN = (((1,), (0,)), ((), ()))
_NT = (((1,), (1,)), ((), ()))


def _dot(a, b, dims=_NN):
    return jax.lax.dot_general(a, b, dims, preferred_element_type=F32)


def _layernorm(x, eps=1e-5):
    d = x - jnp.mean(x, axis=-1, keepdims=True)
    return d * jax.lax.rsqrt(jnp.mean(d * d, axis=-1, keepdims=True) + eps)


def _gelu(x):
    return jax.nn.gelu(x, approximate=True)


def _recip(total):
    r = pl.reciprocal(total, approx=True)
    return r * (2.0 - total * r)


def _softmax(x):
    e = jnp.exp(x - jnp.max(x, axis=-1, keepdims=True))
    return e * _recip(jnp.sum(e, axis=-1, keepdims=True))


def _tree(op, xs):
    while len(xs) > 1:
        xs = [functools.reduce(op, xs[i:i + 2]) for i in range(0, len(xs), 2)]
    return xs[0]


def _kernel(
    x_hbm, mem_ref, wq_hbm, wk_hbm, wv_hbm, wo_hbm, w1_hbm, w2_hbm, w3_hbm, w4_hbm,
    out_hbm,
    x_v, xn_v, h_v, lhs_v, gate_v, out_v, w1_v, w2_v, w3_v, w4_v, wo_v, stored_v, tmp_v,
    kv_v,
    x_sems, w_sems, qkv_sems, out_sem, *wqkv_v, seg,
):
    S, D = x_v.shape
    H, E = len(wqkv_v), LANES
    F = w3_hbm.shape[1]
    M = mem_ref.shape[0]
    n_blk = S // ROWS
    n_col = D // LANES
    DC = D // n_blk

    def aligned_rows(start, align, size, offset=0):
        if not isinstance(start, int):
            start = pl.multiple_of(start, align)
        return pl.ds(start + offset, size)

    def block(i):
        return aligned_rows(i * ROWS, ROWS, ROWS)

    def half(i, p, offset=0, extra=0):
        return aligned_rows(i * ROWS + p * HALF, HALF, HALF + extra, offset)

    def following(i):
        return jnp.minimum(i + 1, n_blk - 1)

    def x_copy(i):
        return pltpu.make_async_copy(x_hbm.at[block(i)], x_v.at[block(i)], x_sems.at[i])

    def qkv_copy(t, c):
        return pltpu.make_async_copy(
            (wq_hbm, wk_hbm, wv_hbm)[t].at[aligned_rows(c * (DC * H), DC * H, DC * H)],
            stored_v.bitcast(BF16).at[t, c, pl.ds(0, DC * H)],
            qkv_sems.at[t * n_blk + c])

    F1 = (WAIT_AT + 1) * FC
    pieces = dict(
        w1=(w1_hbm, w1_v, 0, D, 0, D),
        w2=(w2_hbm, w2_v, 0, D, 0, D),
        w3_early=(w3_hbm, w3_v, 0, D, 0, F1),
        w4_early=(w4_hbm, w4_v, 0, F1, 0, D),
        w3_late=(w3_hbm, w3_v, 0, D, F1, F - F1),
        w4_late=(w4_hbm, w4_v, F1, F - F1, 0, D),
        wo=(wo_hbm, wo_v, 0, H * E, 0, D),
    )

    def weight_copies(names):
        copies = []
        for name in names:
            src, dst, k0, k, n0, n = pieces[name]
            copies += [
                pltpu.make_async_copy(
                    src.at[pl.ds(k0, k), pl.ds(j * LANES, LANES)],
                    dst.bitcast(BF16).at[j, pl.ds(k0, k)],
                    w_sems.at[list(pieces).index(name)])
                for j in range(n0 // LANES, (n0 + n) // LANES)
            ]
        return copies

    def start_weights(*names):
        for c in weight_copies(names):
            c.start()

    def wait_weights(*names):
        for c in weight_copies(names):
            c.wait()

    def weight(ref, k0, k, n0, n):
        tiles = [ref[j, pl.ds(k0 // 2, k // 2), :]
                 for j in range(n0 // LANES, (n0 + n) // LANES)]
        return pltpu.bitcast(jnp.concatenate(tiles, axis=-1), BF16)

    def put_lhs(value):
        lhs_v[...] = pltpu.bitcast(value, U32)

    def get_lhs():
        return pltpu.bitcast(lhs_v[...], BF16)

    x_copy(0).start()
    start_weights("w1")
    x_copy(1).start()

    h_v[pl.ds(0, HALO), :] = jnp.zeros((HALO, D), F32)
    h_v[pl.ds(HALO + S, HALO), :] = jnp.zeros((HALO, D), F32)

    def normalise(rows):
        xn = _layernorm(x_v[rows, :].astype(F32))
        return xn, _layernorm(xn).astype(BF16)

    def stage1(i, carry):
        @pl.when(i == 1)
        def _():
            start_weights("w3_early", "w4_early")

        @pl.when(i + 1 < n_blk)
        def _():
            x_copy(i + 1).wait()

        ln0 = get_lhs()
        xn1, ln1 = normalise(half(i, 1))
        xn2, ln2 = normalise(half(following(i), 0))
        h0 = _gelu(_dot(ln0, weight(w1_v, 0, D, 0, D)))
        h1 = _gelu(_dot(ln1, weight(w1_v, 0, D, 0, D)))
        xn_v[half(i, 1), :] = xn1
        xn_v[half(following(i), 0), :] = xn2
        put_lhs(ln2)
        h_v[half(i, 0, HALO), :] = h0
        h_v[half(i, 1, HALO), :] = h1
        return carry

    x_copy(0).wait()
    xn_v[half(0, 0), :], ln = normalise(half(0, 0))
    put_lhs(ln)
    wait_weights("w1")
    for i in range(2, n_blk):
        x_copy(i).start()
    start_weights("w2")
    jax.lax.fori_loop(0, n_blk, stage1, 0)

    def shifted(i, p):
        parts = []
        for c, shift in enumerate((-1, 1, -2, 2)):
            window = h_v[half(i, p, 0, 2 * HALO), pl.ds(c * D // 4, D // 4)]
            parts.append(window[HALO + shift:HALO + shift + HALF].astype(BF16))
        return jnp.concatenate(parts, axis=-1)

    def relayout(t, c):
        G = H // SUBLANES
        dst = aligned_rows(c * (DC // 2), DC // 2, DC // 2)
        for j0 in range(4):
            tmp_v[t, j0, pl.ds(0, DC * G), :] = stored_v[t, c, pl.ds(j0, DC * G, stride=4), :]
        for j0 in range(4):
            for j1 in range(G):
                w = tmp_v[t, j0, pl.ds(j1, DC, stride=G), :]
                for odd, bits in enumerate((w, w >> 16)):
                    wqkv_v[2 * (4 * j1 + j0) + odd][dst, pl.ds(t * E, E)] = pltpu.bitcast(
                        bits.astype(jnp.uint16), U32)

    def start_qkv(c):
        for t in range(3):
            qkv_copy(t, c).start()

    def stage2(i, carry):
        @pl.when(i + 1 < n_blk)
        def _():
            start_qkv(i + 1)

        @pl.when(i == 2)
        def _():
            start_weights("wo")

        hs0, hs1 = get_lhs(), shifted(i, 1)
        hs2 = shifted(following(i), 0)
        y0 = _dot(hs0, weight(w2_v, 0, D, 0, D)) + xn_v[half(i, 0), :]
        y1 = _dot(hs1, weight(w2_v, 0, D, 0, D)) + xn_v[half(i, 1), :]
        ln0, ln1 = _layernorm(y0).astype(BF16), _layernorm(y1).astype(BF16)
        ln = jnp.concatenate([ln0, ln1], axis=0)
        acc = jnp.concatenate([y0, y1], axis=0)
        for f in range(F // FC):
            w3 = weight(w3_v, 0, D, f * FC, FC)
            if f == 0:
                u = jnp.concatenate([_dot(ln0, w3), _dot(ln1, w3)], axis=0)
            else:
                u = _dot(ln, w3)
            acc = _dot(_gelu(u).astype(BF16), weight(w4_v, f * FC, FC, 0, D)) + acc
            if f == WAIT_AT:
                @pl.when(i == 0)
                def _():
                    wait_weights("w3_late", "w4_late")

                for t in range(3):
                    qkv_copy(t, i).wait()
                for t in range(3):
                    relayout(t, i)
        put_lhs(hs2)
        gate_v[block(i), :] = jax.nn.silu(acc)
        return carry

    put_lhs(shifted(0, 0))
    wait_weights("w2", "w3_early", "w4_early")
    start_weights("w3_late", "w4_late")
    start_qkv(0)
    jax.lax.fori_loop(0, n_blk, stage2, 0)
    wait_weights("wo")

    L = M + seg
    scale = E ** -0.5
    query = jax.lax.broadcasted_iota(jnp.int32, (L - FEW, L), 0)
    query = jnp.where(query < M, query, query + FEW)
    key = jax.lax.broadcasted_iota(jnp.int32, (L - FEW, L), 1)
    mask = (query < M) | (query >= key)
    row = jax.lax.broadcasted_iota(jnp.int32, (FEW, 1), 0)

    def few_key_attention(q, kv_ref):
        def spread(j, c0):
            return jnp.broadcast_to(kv_ref[pl.ds(j, 1), pl.ds(c0, E)], (FEW, E))

        q = q * (scale * LOG2E)
        scores = [jnp.sum(q * spread(j, 0), axis=-1, keepdims=True) for j in range(M + FEW)]
        scores[M + 1:] = [jnp.where(row >= d, scores[M + d], MASKED * LOG2E)
                          for d in range(1, FEW)]
        top = _tree(jnp.maximum, scores)
        e = [jnp.exp2(a - top) for a in scores]
        o = _tree(jnp.add, [a * spread(j, E) for j, a in enumerate(e)])
        return o * _recip(_tree(jnp.add, e))

    def step(s, mem, slot):
        rows = aligned_rows(s * seg, seg, seg)
        tokens = jnp.concatenate([mem, xn_v[rows, :]], axis=0)

        def project(hd, k0, k):
            w = pltpu.bitcast(wqkv_v[hd][pl.ds(k0 // 2, k // 2), :], BF16)
            return _dot(tokens[:, k0:k0 + k], w)

        qkv, prob, heads = [], [], []
        o, done, it = None, 0, 0
        while done < H:
            if it == 0:
                started = project(0, 0, D // 2)
                qkv.append(project(0, D // 2, D // 2) + started)
            elif it < H:
                qkv.append(project(it, 0, D))
            if len(prob) < H and len(prob) <= it - LAG_SCORES:
                t = qkv[len(prob)]
                q = jnp.concatenate([t[:M, :E], t[M + FEW:, :E]], axis=0)
                scores = _dot(q, t[:, E:2 * E], _NT) * scale
                prob.append(_softmax(jnp.where(mask, scores, MASKED)))
            if len(heads) < H and len(heads) <= it - LAG_VALUES:
                hd = len(heads)
                t = qkv[hd]
                pv = _dot(prob[hd], t[:, 2 * E:])
                kv_v[slot, hd] = t[:M + FEW, E:]
                few = few_key_attention(t[M:M + FEW, :E], kv_v.at[slot, hd])
                heads.append(jnp.concatenate([pv[:M], few, pv[M:]], axis=0))
            ready = it + 1 - LAG_OUT if it < H else H - LAG_OUT + (it + 1 - H) * TAIL
            while done + OUT_HEADS <= min(ready, len(heads)):
                part = _dot(jnp.concatenate(heads[done:done + OUT_HEADS], axis=-1),
                            weight(wo_v, done * E, OUT_HEADS * E, 0, D))
                o = part if o is None else part + o
                done += OUT_HEADS
            it += 1
        out = x_v[rows, :].astype(F32) + o[M:] * gate_v[rows, :]
        out_v[rows, :] = out.astype(out_v.dtype)
        return o[:M]

    def steps(i, mem):
        for u in range(UNROLL):
            mem = step(i * UNROLL + u, mem, u)
        rows = aligned_rows(i * (UNROLL * seg), UNROLL * seg, UNROLL * seg)
        pltpu.make_async_copy(out_v.at[rows], out_hbm.at[rows], out_sem).start()
        return mem

    jax.lax.fori_loop(0, S // (UNROLL * seg), steps, mem_ref[...].astype(F32))
    pltpu.make_async_copy(out_v, out_hbm, out_sem).wait()


@functools.partial(jax.jit, static_argnames=("A_seg_len",))
def pallas_recurrent_scan__memory_aug_recurrent_mem_tr__mixer_s_mlp__prompt_kernel(
    A_x: jax.Array,
    A_mem0: jax.Array,
    A_Wq: jax.Array,
    A_Wk: jax.Array,
    A_Wv: jax.Array,
    A_Wo: jax.Array,
    A_seg_len: int,
    B_x: jax.Array,
    B_w1: jax.Array,
    B_w2: jax.Array,
    B_w3: jax.Array,
    B_w4: jax.Array,
):
    del B_x
    B, S, D = A_x.shape
    _, H, E = A_Wq.shape
    M = A_mem0.shape[1]
    F = B_w3.shape[1]
    seg = int(A_seg_len)
    n_blk = S // ROWS
    assert B == 1 and E == LANES and H % SUBLANES == 0 and M % SUBLANES == 0
    assert seg % SUBLANES == 0 and seg > FEW and S % (UNROLL * seg) == 0
    assert S % ROWS == 0 and n_blk > 2 and F % FC == 0 and F > (WAIT_AT + 1) * FC

    def by_column_tile(k, n):
        return pltpu.VMEM((n // LANES, k // 2, LANES), U32)

    words = D // n_blk * H // 2
    hbm = pl.BlockSpec(memory_space=pl.ANY)
    out = pl.pallas_call(
        functools.partial(_kernel, seg=seg),
        out_shape=jax.ShapeDtypeStruct((S, D), A_x.dtype),
        in_specs=[hbm, pl.BlockSpec(memory_space=pltpu.VMEM)] + [hbm] * 8,
        out_specs=hbm,
        scratch_shapes=[
            pltpu.VMEM((S, D), A_x.dtype),
            pltpu.VMEM((S, D), F32),
            pltpu.VMEM((S + 2 * HALO, D), F32),
            pltpu.VMEM((HALF // 2, D), U32),
            pltpu.VMEM((S, D), F32),
            pltpu.VMEM((S, D), A_x.dtype),
            by_column_tile(D, D),
            by_column_tile(D, D),
            by_column_tile(D, F),
            by_column_tile(F, D),
            by_column_tile(H * E, D),
            pltpu.VMEM((3, n_blk, words + SUBLANES, E), U32),
            pltpu.VMEM((3, 4, words // 4 + SUBLANES, E), U32),
            pltpu.VMEM((UNROLL, H, M + FEW, 2 * E), F32),
            pltpu.SemaphoreType.DMA((n_blk,)),
            pltpu.SemaphoreType.DMA((7,)),
            pltpu.SemaphoreType.DMA((3 * n_blk,)),
            pltpu.SemaphoreType.DMA(()),
        ] + [pltpu.VMEM((D // 2, 3 * E), U32)] * H,
        compiler_params=pltpu.CompilerParams(vmem_limit_bytes=124 * 1024 * 1024),
    )(
        A_x.reshape(S, D), A_mem0.reshape(M, D),
        A_Wq.reshape(D * H, E), A_Wk.reshape(D * H, E), A_Wv.reshape(D * H, E),
        A_Wo.reshape(H * E, D), B_w1, B_w2, B_w3, B_w4,
    )
    return out.reshape(B, S, D)
```
